```python
import os as _os
_os.environ.setdefault("JAX_PLATFORMS", "cpu")
import jax
import jax.numpy as jnp

def _softmax(x, axis=-1):
    return jax.nn.softmax(x, axis=axis)
def _gelu(x):
    return jax.nn.gelu(x, approximate=True)
def _silu(x):
    return jax.nn.silu(x)
def _sigmoid(x):
    return jax.nn.sigmoid(x)
def _layernorm(x, axis=-1, eps=1e-5):
    m = jnp.mean(x, axis=axis, keepdims=True)
    v = jnp.var(x, axis=axis, keepdims=True)
    return (x - m) / jnp.sqrt(v + eps)
def _scatter_add(tgt, idx, src, axis=0):
    return tgt.at[idx].add(src)
def _segment_sum(src, seg, n):
    return jax.ops.segment_sum(src, seg, n)
class _Rng:
    def __init__(self, key):
        self._k = key
    def _next(self):
        self._k, sub = jax.random.split(self._k)
        return sub
    def normal(self, shape):
        return jax.random.normal(self._next(), shape, dtype=jnp.bfloat16)
    def randint(self, lo, hi, shape):
        return jax.random.randint(self._next(), shape, lo, hi, dtype=jnp.int32)
    def uniform(self, shape, lo=0.0, hi=1.0):
        return jax.random.uniform(self._next(), shape, jnp.bfloat16, lo, hi)
    def permutation(self, n):
        return jax.random.permutation(self._next(), n)


kernel_name = 'concat_heads__sliding_block_cached__sliding_block_cached__decode'

def setup_inputs():
    _rng = _Rng(jax.random.key(int.from_bytes(__import__("os").urandom(4), "little")))
    _w = (lambda a: (lambda t: t.astype(jnp.bfloat16) if jnp.issubdtype(t.dtype, jnp.floating) else t)(jnp.asarray(a)))
    def _A_setup():
        B, Sq, D = 1, 1, 640
        Hq, Hkv, Sk, Dh = 32, 32, 4096, 192
        assert Hq % Hkv == 0, (Hq, Hkv)
        return {
            "x": _w((lambda *s: _rng.normal(s) * 0.8)(B, Sq, D)),
            "k_cache": _w((lambda *s: _rng.normal(s) * 0.8)(B, Hkv, Sk, Dh)),
            "v_cache": _w((lambda *s: _rng.normal(s) * 0.05)(B, Hkv, Sk, Dh)),
            "wq": _w((lambda *s: _rng.normal(s) * 0.8)(D, Hq * Dh) * (D ** -0.5)),
            "wo": _w((lambda *s: _rng.normal(s) * 0.05)(Hq * Dh, D) * ((Hq * Dh) ** -0.5)),
        }
    _A_in = _A_setup()

    def _B_setup():
        B, Sq, D = 1, 1, 640
        Hq, Hkv, Sk, Dh = 32, 32, 4096, 192
        assert Hq % Hkv == 0, (Hq, Hkv)
        return {
            "x": _w((lambda *s: _rng.normal(s) * 0.8)(B, Sq, D)),
            "k_cache": _w((lambda *s: _rng.normal(s) * 0.8)(B, Hkv, Sk, Dh)),
            "v_cache": _w((lambda *s: _rng.normal(s) * 0.05)(B, Hkv, Sk, Dh)),
            "wq": _w((lambda *s: _rng.normal(s) * 0.8)(D, Hq * Dh) * (D ** -0.5)),
            "wo": _w((lambda *s: _rng.normal(s) * 0.05)(Hq * Dh, D) * ((Hq * Dh) ** -0.5)),
        }
    _B_in = _B_setup()

    return {
        "A_x": _A_in["x"],
        "A_k_cache": _A_in["k_cache"],
        "A_v_cache": _A_in["v_cache"],
        "A_wq": _A_in["wq"],
        "A_wo": _A_in["wo"],
        "B_x": _B_in["x"],
        "B_k_cache": _B_in["k_cache"],
        "B_v_cache": _B_in["v_cache"],
        "B_wq": _B_in["wq"],
        "B_wo": _B_in["wo"],
    }

def reference(A_x, A_k_cache, A_v_cache, A_wq, A_wo, B_x, B_k_cache, B_v_cache, B_wq, B_wo):
    def _A_ref(x, k_cache, v_cache, wq, wo):
        B, Sq, D = x.shape
        Hq, Dh = 32, 192
        Hkv, Sk = k_cache.shape[1], k_cache.shape[2]
        W = min(4096, max(256, Sk // 4))
        rep = Hq // Hkv
        q = (lambda x, *d: x.transpose(*d))((x @ wq).reshape(B, Sq, Hq, Dh), 0, 2, 1, 3)
        k = jnp.repeat(k_cache[:, :, Sk - W:, :], rep, axis=1)
        v = jnp.repeat(v_cache[:, :, Sk - W:, :], rep, axis=1)
        scores = jnp.einsum("bhqd,bhkd->bhqk", q, k) * (Dh ** -0.5)
        p = _softmax(scores, axis=-1)
        o = jnp.einsum("bhqk,bhkd->bhqd", p, v)
        return (lambda x, *d: x.transpose(*d))(o, 0, 2, 1, 3).reshape(B, Sq, Hq * Dh) @ wo

    def _B_ref(x, k_cache, v_cache, wq, wo):
        B, Sq, D = x.shape
        Hq, Dh = 32, 192
        Hkv, Sk = k_cache.shape[1], k_cache.shape[2]
        W = min(4096, max(256, Sk // 4))
        rep = Hq // Hkv
        q = (lambda x, *d: x.transpose(*d))((x @ wq).reshape(B, Sq, Hq, Dh), 0, 2, 1, 3)
        k = jnp.repeat(k_cache[:, :, Sk - W:, :], rep, axis=1)
        v = jnp.repeat(v_cache[:, :, Sk - W:, :], rep, axis=1)
        scores = jnp.einsum("bhqd,bhkd->bhqk", q, k) * (Dh ** -0.5)
        p = _softmax(scores, axis=-1)
        o = jnp.einsum("bhqk,bhkd->bhqd", p, v)
        return (lambda x, *d: x.transpose(*d))(o, 0, 2, 1, 3).reshape(B, Sq, Hq * Dh) @ wo

    a = _A_ref(A_x, A_k_cache, A_v_cache, A_wq, A_wo)
    b = _B_ref(B_x, B_k_cache, B_v_cache, B_wq, B_wo)
    return jnp.concatenate([a, b], axis=-1)
```

```python
import jax, jax.numpy as jnp
from jax import lax
import jax.experimental.pallas as pl
import jax.experimental.pallas.tpu as pltpu
bf, f32 = jnp.bfloat16, jnp.float32
D, H, DH, SK, W = 640, 32, 192, 4096, 1024
G = 8
GR = G * DH
NG = H // G

def kern(ax, ak, av, awq, awo, bx, bk, bv, bwq, bwo, o_ref, xs, kb, vb, qb, ob, sems):
    X = (ax, bx); K = (ak, bk); V = (av, bv); WQ = (awq, bwq); WO = (awo, bwo)
    cp = {}
    n = [0]
    def mk(key, s, d):
        cp[key] = pltpu.make_async_copy(s, d, sems.at[n[0]]); n[0] += 1
        cp[key].start()
    for b in range(2):
        mk(("q", b), WQ[b], qb.at[b])
        mk(("x", b), X[b].at[0], xs.at[b])
    for b in range(2):
        for g in range(NG):
            rows = pl.ds(g*GR, GR)
            mk(("k", b, g), K[b].at[rows, pl.ds(SK-W, W)], kb.at[b, rows])
            mk(("v", b, g), V[b].at[rows, pl.ds(SK-W, W)], vb.at[b, rows])
            mk(("o", b, g), WO[b].at[rows], ob.at[b, rows])
    row = lax.broadcasted_iota(jnp.int32, (G, GR), 0)
    col = lax.broadcasted_iota(jnp.int32, (G, GR), 1)
    own = (col >= row*DH) & (col < (row+1)*DH)
    for b in range(2):
        cp["x", b].wait(); cp["q", b].wait()
        x8 = jnp.broadcast_to(xs[b].astype(f32), (G, D)).astype(bf)
        acc = jnp.zeros((G, D), f32)
        for g in range(NG):
            rows = pl.ds(g*GR, GR)
            q = jnp.dot(x8, qb[b, :, g*GR:(g+1)*GR], preferred_element_type=f32)
            q = jnp.where(own, q, 0.0).astype(bf)
            cp["k", b, g].wait()
            s = jnp.dot(q, kb[b, rows], preferred_element_type=f32) * (DH ** -0.5)
            m = jnp.max(s, axis=-1, keepdims=True)
            e = jnp.exp(s - m)
            p = (e / jnp.sum(e, axis=-1, keepdims=True)).astype(bf)
            cp["v", b, g].wait()
            o = lax.dot_general(p, vb[b, rows], (((1,), (1,)), ((), ())), preferred_element_type=f32)
            o = jnp.where(own, o, 0.0).astype(bf)
            cp["o", b, g].wait()
            acc = acc + jnp.dot(o, ob[b, rows], preferred_element_type=f32)
        o_ref[0, :, b*D:(b+1)*D] = jnp.sum(acc, axis=0, keepdims=True).astype(bf)

@jax.jit
def pallas_concat_heads__sliding_block_cached__sliding_block_cached__decode_kernel(A_x, A_k_cache, A_v_cache, A_wq, A_wo, B_x, B_k_cache, B_v_cache, B_wq, B_wo):
    ax, ak, av, awq, awo, bx, bk, bv, bwq, bwo = A_x, A_k_cache, A_v_cache, A_wq, A_wo, B_x, B_k_cache, B_v_cache, B_wq, B_wo
    t = lambda a: jnp.swapaxes(a, 2, 3).reshape(H*DH, SK)
    return pl.pallas_call(
        kern,
        out_shape=jax.ShapeDtypeStruct((1,1,2*D), bf),
        in_specs=[pl.BlockSpec(memory_space=pltpu.HBM)]*10,
        scratch_shapes=[pltpu.VMEM((2,1,D), bf), pltpu.VMEM((2,H*DH,W), bf), pltpu.VMEM((2,H*DH,W), bf),
                        pltpu.VMEM((2,D,H*DH), bf), pltpu.VMEM((2,H*DH,D), bf), pltpu.SemaphoreType.DMA((4+6*NG,))],
        compiler_params=pltpu.CompilerParams(vmem_limit_bytes=120*1024*1024, disable_bounds_checks=True, disable_semaphore_checks=True),
        name="k0",
    )(ax, t(ak), t(av), awq, awo, bx, t(bk), t(bv), bwq, bwo)
```

```python
import jax, jax.numpy as jnp
from jax import lax
import jax.experimental.pallas as pl
import jax.experimental.pallas.tpu as pltpu
bf, f32 = jnp.bfloat16, jnp.float32
D, H, DH, SK, W = 640, 32, 192, 4096, 1024
R = H * DH
T = 128
NT = R // T
GT = 8 * DH // T
KA, KB = 96, 64
WA, WB = 15, 2048
NS = 16
U = NT // NS

def loop(lo, hi, fn):
    if isinstance(hi, int) and isinstance(lo, int) and hi - lo <= 1:
        if hi - lo == 1: fn(lo)
    else: lax.fori_loop(lo, hi, lambda i, c: (fn(i), c)[1], 0)
def mo(x, n): return x if isinstance(x, int) else pl.multiple_of(x, n)
def div(x, n): return x // n if isinstance(x, int) else lax.div(x, jnp.int32(n))
def rem(x, n): return x % n if isinstance(x, int) else lax.rem(x, jnp.int32(n))
def P(s): return [(int(x[0], 36), int(x[1])) for x in s.split()]
def iota(shape, d): return lax.broadcasted_iota(jnp.int32, shape, d)

def make(L=4, kvp="10 71", kw=512, span=16, order="csb", ksep=True, wp="10 41 31 10 31 31", ww=32, wsep=True, tail=(8, 3, 2, 1, 1), peel=1, nocompute=False, manual_out=False, cp=None, ev=2, tw=128, nvpu=4, tp='10 41 31', wx=False):
    assert sum(tail) == WA
    def kern(ax, ak, av, awq, awo, bx, bk, bv, bwq, bwo, o_ref, xs, kb, vb, qb, ob, xe, qs, ss, os_, es, ec, sems, *rest):
        X, K, V, WQ, WO = (ax, bx), (ak, bk), (av, bv), (awq, bwq), (awo, bwo)
        def sweep(pat, sep, a0, n, go):
            pat = P(pat); per = sum(m for m, _ in pat); n0 = sum(m for m, p in pat if p == 0)
            assert n % per == 0
            pos = [0, n // per * n0]; a = 0
            for i in range(n // per):
                for m, p in pat:
                    go(a0 + (pos[p] if sep else a), m, p); pos[p] += m; a += m
        def w_copy(src, dst, br, a, m, r, nr, sem):
            rows = pl.ds(mo(r, 32), nr)
            return pltpu.make_async_copy(src[br].at[pl.ds(a, m), rows], dst.at[pl.ds(br * WA + a, m), rows], sems.at[sem])
        wps = wp.split(",")
        def w_round(src, dst, br, jj, sem):
            for i, pat in enumerate(wps):
                j = jj * len(wps) + i
                if wx and src is WQ: j = (j & 33) | ((j & 2) << 3) | ((j >> 1) & 14)
                sweep(pat, wsep, 0, WA, lambda a, m, p: w_copy(src, dst, br, a, m, j * ww, ww, sem).start(priority=p))
        nr = T // ww // len(wps)
        def issue_q(br, t): loop(t * nr, (t + 1) * nr, lambda j: w_round(WQ, qb, br, j, br))
        def issue_o(br, t): loop(t * nr, (t + 1) * nr, lambda j: w_round(WO, ob, br, j, 7 + br * NS + t))
        def issue_kv(src, dst, sem):
            ns = KA // span; nc = W // kw; n = 8 * ns * nc // NS
            assert n * NS == 8 * ns * nc and ns * span == KA
            def f(br, t):
                def one(j):
                    c = rem(j, nc); j2 = div(j, nc)
                    if order == "csb": s, b = rem(j2, ns), div(j2, ns)
                    elif order == "cbs": b, s = j2 & 7, j2 >> 3
                    elif order == "cbsx":
                        b, s = j2 & 7, j2 >> 3
                        b = (b & 4) | ((b & 1) << 1) | ((b >> 1) & 1)
                    elif order == "c2sb":
                        s, b = rem(j2 >> 1, ns), div(j2 >> 1, ns)
                        b = ((b & 2) << 1) | ((j2 & 1) << 1) | (b & 1)
                    elif order == "c4sb":
                        s, b = rem(j2 >> 2, ns), div(j2 >> 2, ns)
                        b = ((j2 & 3) << 1) | b
                    rows = pl.ds(mo(b * 8, 8), 8)
                    def go(a, m, p):
                        pltpu.make_async_copy(src[br].at[pl.ds(a, m), rows, pl.ds(mo(SK - W + c * kw, T), kw)],
                                              dst.at[pl.ds(br * KA + a, m), rows, pl.ds(mo(c * kw, T), kw)], sems.at[sem + br]).start(priority=p)
                    sweep(kvp, ksep, s * span, span, go)
                loop(t * n, (t + 1) * n, one)
            return f
        stages = [issue_q, issue_kv(K, kb, 2), issue_kv(V, vb, 4), issue_o]
        def issue(lo, hi, i):
            arrs = [a for a in range(8) if a * NS < hi and (a + 1) * NS > lo]
            for a in arrs:
                f = lambda a=a: stages[a // 2](a % 2, i - a * NS)
                if len(arrs) == 1: f()
                else: pl.when((i >= a * NS) & (i < (a + 1) * NS))(f)
        def wait(buf, sem): pltpu.make_async_copy(buf, buf, sems.at[sem]).wait()

        off = NS + L
        for j in range(peel): w_round(WQ, qb, 0, j, 0)
        loop(peel, NS * nr, lambda j: w_round(WQ, qb, 0, j, 0))
        for b in range(2): pltpu.make_async_copy(X[b].at[0], xs.at[b], sems.at[6]).start()
        loop(0, L * nr, lambda j: w_round(WQ, qb, 1, j, 1))
        ss[...] = jnp.zeros(ss.shape, f32)
        qs[...] = jnp.zeros(qs.shape, f32)
        wait(xs, 6)
        def spread_x(br):
            own = (iota((D // 8, D), 1) >> 3) == iota((D // 8, D), 0)
            sel = jnp.where((iota((D, T), 0) & 7) == (iota((D, T), 1) & 7), 1.0, 0.0).astype(bf)
            xe[br] = jnp.dot(jnp.where(own, xs[br].astype(f32), 0.0).astype(bf), sel, preferred_element_type=f32)
        loop(0, 2, spread_x)
        def stage(s, buf, na, compute):
            base = 2 * NS * s + off
            def step(c):
                issue(base, base + 2 * NS, base + c)
                br = div(c, NS)
                pl.when(rem(c, NS) == 0)(lambda: wait(buf.at[pl.ds(br * na, na)], 2 * s + br))
                if not nocompute: compute(br, rem(c, NS))
            loop(0, 2 * NS, step)
        def c_q(br, t):
            own = (iota((16, T), 1) >> 3) == iota((16, T), 0)
            ls, ws = [], []
            for j in range(5):
                r = t * 5 + j
                ls.append(jnp.where(own, xe[br, pl.ds(r, 1)], 0.0))
                us = [r * 3 + i for i in range(3)]
                ws.append(jnp.concatenate([qb[br * WA + (u >> 4), pl.ds(mo((u & 15) * T, T), T)] for u in us], axis=1))
            q = jnp.dot(jnp.concatenate(ls, axis=1).astype(bf), jnp.concatenate(ws, axis=0), preferred_element_type=f32)
            for i in range(3): qs[br, i * 16:(i + 1) * 16] += q[:, i * T:(i + 1) * T]
        stage(0, qb, WA, c_q)
        def own_head(t):
            row = iota((8, U * T), 0); col = iota((8, U * T), 1) + rem(t * U, GT) * T
            return (col >= row * DH) & (col < (row + 1) * DH)
        def c_s(br, t):
            k = kb[pl.ds(br * KA + t * (KA // NS), KA // NS)].reshape(U * T, W)
            q = jnp.concatenate([qs[br, pl.ds(t * U + j, 1)] for j in range(U)], axis=1)
            q = jnp.where(own_head(t), q, 0.0).astype(bf)
            ss[br, div(t * U, GT)] += jnp.dot(q, k, preferred_element_type=f32)
        stage(1, kb, KA, c_s)
        def c_o(br, t):
            g = div(t * U, GT)
            @pl.when(rem(t * U, GT) == 0)
            def _():
                s = ss[br, g] * (DH ** -0.5)
                e = jnp.exp(s - jnp.max(s, axis=-1, keepdims=True))
                ss[br, g] = e / jnp.sum(e, axis=-1, keepdims=True)
            v = vb[pl.ds(br * KA + t * (KA // NS), KA // NS)].reshape(U * T, W)
            o = lax.dot_general(ss[br, g].astype(bf), v, (((1,), (1,)), ((), ())), preferred_element_type=f32)
            o = jnp.sum(jnp.where(own_head(t), o, 0.0), axis=0, keepdims=True)
            for j in range(U): os_[pl.ds(br * NT + t * U + j, 1)] = o[:, j * T:(j + 1) * T]
        stage(2, vb, KA, c_o)
        if not nocompute:
            col = iota((T, D), 1)
            lo = (iota((T, D), 0) >> 3) * 40
            sel = jnp.where((col >= lo) & (col < lo + 40) & ((col & 7) == (iota((T, D), 0) & 7)), 1.0, 0.0).astype(bf)
            e = jnp.dot(os_[...].astype(bf), sel, preferred_element_type=f32)
            for j in range(5): es[pl.ds(j, 2 * NT, stride=5)] = e[:, j * T:(j + 1) * T]
        base = 6 * NS + off
        last = 8 * NS - 1
        d = iota((8, T), 0) - (iota((8, T), 1) >> 3) + 15
        for _ in range(4): d = jnp.where(d >= 5, d - 5, d)
        d = jnp.where(iota((8, T), 0) < 5, d, -1)
        def project(acc, br, j, a0, n, sem):
            w = ob.at[pl.ds(br * WA + a0, n), pl.ds(mo(j * T, T), T)]
            if nocompute:
                wait(w, sem); return acc
            ls = []
            for a in range(a0, a0 + n):
                u = a * 16 + j
                ls.append(jnp.where(d == rem(u, 5), es[pl.ds(br * 5 * NT + u, 1)], 0.0))
            l = jnp.concatenate(ls, axis=1).astype(bf)
            wait(w, sem)
            return acc + jnp.dot(l, w[...].reshape(n * T, T), preferred_element_type=f32)
        ov = rest[0] if manual_out else o_ref
        def store(br, acc):
            ov[0, :, br * D:(br + 1) * D] = jnp.concatenate([acc[c:c + 1] for c in range(5)], axis=1).astype(bf)
        def out_copy(br): return pltpu.make_async_copy(ov.at[:, :, pl.ds(br * D, D)], o_ref.at[:, :, pl.ds(br * D, D)], sems.at[br])
        def issue_tail():
            a0 = 0
            for i, n in enumerate(tail):
                sem = 6 + 2 * NS + i
                if i == 0:
                    for j in range(T // ww):
                        sweep(tp or f"10 {(n-1)//2:x}1 10 {n-2-(n-1)//2:x}1", True, 0, n, lambda a, m, p: w_copy(WO, ob, 1, a, m, WB - T + j * ww, ww, sem).start(priority=p))
                else:
                    for j in range(T // tw): w_copy(WO, ob, 1, a0, n, WB - T + j * tw, tw, sem).start(priority=1)
                a0 += n
        def c_out(c, acc):
            ct = (last - base) * ev
            assert ct < 2 * NS - 1
            pl.when((c < ct) & (rem(c, ev) == 0))(lambda: issue(base, last, base + div(c, ev)))
            pl.when(c == ct)(issue_tail)
            @pl.when(c == NS)
            def _():
                store(0, acc)
                if manual_out: out_copy(0).start()
            return project(jnp.where(c == NS, 0.0, acc), div(c, NS), rem(c, NS), 0, WA, 7 + c)
        nv = sum(tail[len(tail) - nvpu:])
        for i in range(nv):
            u = 5 * NT + (WA - nv + i) * 16 + NS - 1
            ec[i] = jnp.broadcast_to(es[pl.ds(u, 1)], (T, T)).T
        acc = lax.fori_loop(0, 2 * NS - 1, c_out, jnp.zeros((8, T), f32))
        if manual_out: out_copy(0).wait()
        a0 = 0
        for i, n in enumerate(tail[:len(tail) - nvpu]):
            acc = project(acc, 1, NS - 1, a0, n, 6 + 2 * NS + i); a0 += n
        if nvpu:
            part = [jnp.where(iota((8, T), 0) == c, acc, 0.0) for c in range(5)]
            for i in range(len(tail) - nvpu, len(tail)):
                n = tail[i]
                wait(ob.at[pl.ds(WA + a0, n), pl.ds(WB - T, T)], 6 + 2 * NS + i)
                for a in range(a0, a0 + n):
                    y = ob[WA + a, WB - T:].astype(f32) * ec[a - (WA - nv)]
                    for k in range(16):
                        c = (a * 16 + NS - 1 + k) % 5
                        part[c] = part[c] + y[k * 8:(k + 1) * 8]
                a0 += n
            ov[0, :, D:] = jnp.concatenate([jnp.sum(p, axis=0, keepdims=True) for p in part], axis=1).astype(bf)
        else: store(1, acc)
        if manual_out:
            out_copy(1).start(); out_copy(1).wait()

    def f(ax, ak, av, awq, awo, bx, bk, bv, bwq, bwo):
        t = lambda a: jnp.swapaxes(a, 2, 3).reshape(KA, KB, SK)
        w = lambda a: a.reshape(a.shape[0] // 8, 8, a.shape[1] // T, T).transpose(0, 2, 1, 3).reshape(WA, WB, T)
        kw_ = dict(vmem_limit_bytes=120*1024*1024, disable_bounds_checks=True, disable_semaphore_checks=True); kw_.update(cp or {})
        return pl.pallas_call(
            kern,
            out_shape=jax.ShapeDtypeStruct((1,1,2*D), bf),
            in_specs=[pl.BlockSpec(memory_space=pltpu.HBM)]*10,
            out_specs=pl.BlockSpec(memory_space=pltpu.HBM if manual_out else pltpu.VMEM),
            scratch_shapes=[pltpu.VMEM((2,1,D), bf), pltpu.VMEM((2*KA,KB,W), bf), pltpu.VMEM((2*KA,KB,W), bf),
                            pltpu.VMEM((2*WA,WB,T), bf), pltpu.VMEM((2*WA,WB,T), bf),
                            pltpu.VMEM((2,D//8,T), f32), pltpu.VMEM((2,NT,T), f32), pltpu.VMEM((2,4,8,W), f32), pltpu.VMEM((2*NT,T), f32), pltpu.VMEM((10*NT,T), f32), pltpu.VMEM((8,T,T), f32),
                            pltpu.SemaphoreType.DMA((6+2*NS+len(tail),))] + ([pltpu.VMEM((1,1,2*D), bf)] if manual_out else []),
            compiler_params=pltpu.CompilerParams(**kw_),
            name="k3",
        )(ax, t(ak), t(av), w(awq), w(awo), bx, t(bk), t(bv), w(bwq), w(bwo))
    return f


@jax.jit
def pallas_concat_heads__sliding_block_cached__sliding_block_cached__decode_kernel(
        A_x, A_k_cache, A_v_cache, A_wq, A_wo, B_x, B_k_cache, B_v_cache, B_wq, B_wo):
    return make(kvp='10 41 31', span=24, order='c2sb')(A_x, A_k_cache, A_v_cache, A_wq, A_wo, B_x, B_k_cache, B_v_cache, B_wq, B_wo)
```

```python
import jax
import jax.numpy as jnp
from jax import lax
import jax.experimental.pallas as pl
import jax.experimental.pallas.tpu as pltpu

BF16, F32 = jnp.bfloat16, jnp.float32

D, H, DH, SK = 640, 32, 192, 4096
W = min(4096, max(256, SK // 4))
T = 128
NT = H * DH // T
NC = D // T
GROUP = 8 * DH

KV_BLOCKS, KV_ROWS = 96, 64
W_BLOCKS, W_ROWS = 15, 2048
PIECE = 32

WQ, K, V, WO = 0, 2, 4, 6
ROUNDS = 64
LAG = 12
SETTLE = 8

STEPS = 16
TILES = NT // STEPS
TAIL_STEP = 26
TAIL_MXU = 8
TAIL_VPU = (3, 2, 1, 1)

SEM_X, SEM_WO = 10, 11
SEM_TAIL = SEM_WO + 2 * STEPS


def _loop(lo, hi, fn):
    lax.fori_loop(lo, hi, lambda i, carry: (fn(i), carry)[1], 0)


def _ds(start, size):
    if not isinstance(start, int):
        start = pl.multiple_of(start, size)
    return pl.ds(start, size)


def _iota(shape, axis):
    return lax.broadcasted_iota(jnp.int32, shape, axis)


def _ones_where(mask):
    return jnp.where(mask, 1.0, 0.0).astype(BF16)


def _kernel(a_x, a_k, a_v, a_wq, a_wo, b_x, b_k, b_v, b_wq, b_wo, out_ref,
            x_buf, k_buf, v_buf, wq_buf, wo_buf, x_rows, q_buf, p_buf, o_buf,
            o_rows, o_cols, sems):
    src = (a_wq, b_wq, a_k, b_k, a_v, b_v, a_wo, b_wo)
    dst = (wq_buf, wq_buf, k_buf, k_buf, v_buf, v_buf, wo_buf, wo_buf)

    def weight_copy(t, block, n, rows, sem):
        return pltpu.make_async_copy(
            src[t].at[pl.ds(block, n), rows],
            dst[t].at[pl.ds(t % 2 * W_BLOCKS + block, n), rows],
            sems.at[sem])

    def units(t):
        return 4 if K <= t < WO else 3

    def start_unit(t, rnd, unit, queue):
        if K <= t < WO:
            half = rnd >> 5
            rows = _ds((((rnd >> 1) & 6) | ((rnd >> 4) & 1)) * 8, 8)
            col = (unit & 1) * (W // 2)
            block = half * 48 + (rnd & 3) * 12 + (unit >> 1) * 6
            spans = ((1, 2), (3, 3)) if queue else ((0, 1),)
            for first, n in spans:
                pltpu.make_async_copy(
                    src[t].at[pl.ds(block + first, n), rows,
                              _ds(SK - W + col, W // 2)],
                    dst[t].at[pl.ds(t % 2 * KV_BLOCKS + block + first, n), rows,
                              _ds(col, W // 2)],
                    sems.at[2 * t - 2 + half]).start(priority=queue)
        else:
            rows = _ds(rnd * PIECE, PIECE)
            sem = t if t < K else SEM_WO + t % 2 * STEPS + (rnd >> 2)
            spans = (((3 + 4 * unit, 2), (5 + 4 * unit, 2)) if queue
                     else ((unit, 1),))
            for block, n in spans:
                weight_copy(t, block, n, rows, sem).start(priority=queue)

    def first_round(t, rnd):
        for unit in range(units(t)):
            if t and units(t) == units(t - 1):
                start_unit(t - 1, ROUNDS - LAG // units(t) + rnd, unit, 0)
            elif t:
                start_unit(t - 1, ROUNDS - units(t) + unit, rnd, 0)
            start_unit(t, rnd, unit, 1)

    def later_round(t, rnd):
        for unit in range(units(t)):
            start_unit(t, rnd - LAG // units(t), unit, 0)
            start_unit(t, rnd, unit, 1)

    def issue(lo, hi, first, last):
        clip_lo, clip_hi = ((max, min) if isinstance(first, int)
                            else (jnp.maximum, jnp.minimum))
        for t in range(len(src)):
            base, split = t * ROUNDS, LAG // units(t)
            for r0, r1, fn in ((0, split, first_round),
                               (split, ROUNDS, later_round)):
                if base + r1 > lo and base + r0 < hi:
                    _loop(clip_lo(first - base, r0), clip_hi(last - base, r1),
                          lambda rnd, fn=fn, t=t: fn(t, rnd))

    def issue_tail():
        copies = [(block, 2, _ds(W_ROWS - T + piece * PIECE, PIECE), SEM_TAIL - 1)
                  for piece in range(T // PIECE)
                  for block in range(0, TAIL_MXU, 2)]
        block = TAIL_MXU
        for batch, n in enumerate(TAIL_VPU):
            copies += [(block + i, 1, _ds(W_ROWS - T, T), SEM_TAIL + batch)
                       for i in range(n)]
            block += n
        for i in range(LAG):
            start_unit(WO + 1, ROUNDS - 8 + i // 3, i % 3, 0)
            for copy in copies[i * len(copies) // LAG:
                               (i + 1) * len(copies) // LAG]:
                weight_copy(WO + 1, *copy).start(priority=1)

    def wait(filled, sem):
        pltpu.make_async_copy(filled, filled, sems.at[sem]).wait()

    def stage(lo, hi, round_at, buf, parts, sem, compute):
        steps = 2 * STEPS // parts
        size = buf.shape[0] // parts

        def step(c):
            issue(lo, hi, round_at(c), round_at(c + 1))
            part = lax.div(c, steps)
            pl.when(lax.rem(c, steps) == 0)(
                lambda: wait(buf.at[pl.ds(part * size, size)], sem + part))
            compute(lax.div(c, STEPS), lax.rem(c, STEPS))

        _loop(0, 2 * STEPS, step)

    q_at = ROUNDS + SETTLE
    s_at = K * ROUNDS + ROUNDS // 2 + SETTLE
    o_at = V * ROUNDS + ROUNDS // 2 + SETTLE
    out_at = WO * ROUNDS + ROUNDS // 2 + SETTLE
    tail_at = len(src) * ROUNDS - 4

    first_round(WQ, 0)
    issue(1, ROUNDS, 1, ROUNDS)
    for br, x in enumerate((a_x, b_x)):
        pltpu.make_async_copy(x.at[0], x_buf.at[br], sems.at[SEM_X]).start()
    issue(ROUNDS, q_at, ROUNDS, q_at)
    q_buf[...] = jnp.zeros(q_buf.shape, F32)
    p_buf[...] = jnp.zeros(p_buf.shape, F32)
    wait(x_buf, SEM_X)

    def spread_x(br):
        own = (_iota((D // 8, D), 1) >> 3) == _iota((D // 8, D), 0)
        x = jnp.where(own, x_buf[br].astype(F32), 0.0).astype(BF16)
        spread = _ones_where((_iota((D, T), 0) & 7) == (_iota((D, T), 1) & 7))
        x_rows[br] = jnp.dot(x, spread, preferred_element_type=F32)

    _loop(0, 2, spread_x)

    def project_q(br, step):
        diagonal = (_iota((16, T), 1) >> 3) == _iota((16, T), 0)
        n = D // 8 // STEPS
        lhs, rhs = [], []
        for r in (step * n + i for i in range(n)):
            lhs.append(jnp.where(diagonal, x_rows[br, pl.ds(r, 1)], 0.0))
            rhs.append(jnp.concatenate(
                [wq_buf[br * W_BLOCKS + (u >> 4), _ds((u & 15) * T, T)]
                 for u in (3 * r, 3 * r + 1, 3 * r + 2)], axis=1))
        q = jnp.dot(jnp.concatenate(lhs, axis=1).astype(BF16),
                    jnp.concatenate(rhs, axis=0), preferred_element_type=F32)
        for i in range(3):
            q_buf[br, 16 * i:16 * (i + 1)] += q[:, i * T:(i + 1) * T]

    stage(q_at, s_at, lambda c: q_at + 4 * c - 2 * jnp.maximum(c - STEPS, 0),
          wq_buf, 2, 0, project_q)

    def own_head(step):
        row = _iota((8, TILES * T), 0)
        col = _iota((8, TILES * T), 1) + lax.rem(step * TILES * T, GROUP)
        return (col >= row * DH) & (col < (row + 1) * DH)

    def cache_rows(buf, br, step):
        n = KV_BLOCKS // STEPS
        return buf[pl.ds(br * KV_BLOCKS + step * n, n)].reshape(TILES * T, W)

    def scores(br, step):
        q = jnp.concatenate([q_buf[br, pl.ds(step * TILES + i, 1)]
                             for i in range(TILES)], axis=1)
        q = jnp.where(own_head(step), q, 0.0).astype(BF16)
        group = lax.div(step * TILES * T, GROUP)
        p_buf[br, group] += jnp.dot(q, cache_rows(k_buf, br, step),
                                    preferred_element_type=F32)

        @pl.when(lax.rem((step + 1) * TILES * T, GROUP) == 0)
        def _():
            s = p_buf[br, group] * (DH ** -0.5)
            e = jnp.exp(s - jnp.max(s, axis=-1, keepdims=True))
            p_buf[br, group] = e / jnp.sum(e, axis=-1, keepdims=True)

    stage(s_at, o_at, lambda c: s_at + 4 * c, k_buf, 4, 2, scores)

    def values(br, step):
        p = p_buf[br, lax.div(step * TILES * T, GROUP)].astype(BF16)
        o = lax.dot_general(p, cache_rows(v_buf, br, step),
                            (((1,), (1,)), ((), ())), preferred_element_type=F32)
        o = jnp.sum(jnp.where(own_head(step), o, 0.0), axis=0, keepdims=True)
        for i in range(TILES):
            o_buf[pl.ds(br * NT + step * TILES + i, 1)] = o[:, i * T:(i + 1) * T]

    stage(o_at, out_at, lambda c: o_at + 4 * c, v_buf, 4, 6, values)

    row, col = _iota((T, D), 0), _iota((T, D), 1)
    first = (row >> 3) * (8 * NC)
    spread = _ones_where((col >= first) & (col < first + 8 * NC)
                         & ((col & 7) == (row & 7)))
    o = jnp.dot(o_buf[...].astype(BF16), spread, preferred_element_type=F32)
    for i in range(NC):
        o_rows[i] = o[:, i * T:(i + 1) * T]

    row = _iota((8, T), 0)
    phase = row - (_iota((8, T), 1) >> 3) + 3 * NC
    for _ in range(3):
        phase = jnp.where(phase >= NC, phase - NC, phase)
    phase = jnp.where(row < NC, phase, -1)

    def project_out(acc, br, group, blocks, sem):
        lhs = [None] * blocks
        for i in range(NC):
            u = i * STEPS + group
            plane, r = lax.rem(u, NC), br * NT + lax.div(u, NC)
            for block in range(i, blocks, NC):
                o = o_rows[plane, pl.ds(r + block // NC * STEPS, 1)]
                lhs[block] = jnp.where(phase == plane, o, 0.0)
        lhs = jnp.concatenate(lhs, axis=1).astype(BF16)
        wo = wo_buf.at[pl.ds(br * W_BLOCKS, blocks), _ds(group * T, T)]
        wait(wo, sem)
        return acc + jnp.dot(lhs, wo[...].reshape(blocks * T, T),
                             preferred_element_type=F32)

    def out_step(c, acc):
        rate = pl.cdiv((tail_at - out_at) * 16, TAIL_STEP)
        issue(out_at, tail_at,
              jnp.minimum(out_at + ((c * rate) >> 4), tail_at),
              jnp.minimum(out_at + (((c + 1) * rate) >> 4), tail_at))
        pl.when(c == TAIL_STEP)(issue_tail)

        @pl.when(c < sum(TAIL_VPU))
        def _():
            u = (TAIL_MXU + c + 1) * STEPS - 1
            o = o_rows[lax.rem(u, NC), pl.ds(NT + lax.div(u, NC), 1)]
            o_cols[c] = jnp.broadcast_to(o, (T, T)).T

        @pl.when(c == STEPS)
        def _():
            out_ref[0, :, :D] = jnp.concatenate(
                [acc[i:i + 1] for i in range(NC)], axis=1).astype(BF16)

        return project_out(jnp.where(c == STEPS, 0.0, acc), lax.div(c, STEPS),
                           lax.rem(c, STEPS), W_BLOCKS, SEM_WO + c)

    acc = lax.fori_loop(0, 2 * STEPS - 1, out_step, jnp.zeros((8, T), F32))
    acc = project_out(acc, 1, STEPS - 1, TAIL_MXU, SEM_TAIL - 1)

    sums = [jnp.where(row == i, acc, 0.0) for i in range(NC)]
    first = TAIL_MXU
    for batch, n in enumerate(TAIL_VPU):
        wait(wo_buf.at[pl.ds(W_BLOCKS + first, n), _ds(W_ROWS - T, T)],
             SEM_TAIL + batch)
        for block in range(first, first + n):
            prod = (wo_buf[W_BLOCKS + block, W_ROWS - T:].astype(F32)
                    * o_cols[block - TAIL_MXU])
            for i in range(T // 8):
                sums[((block + 1) * STEPS - 1 + i) % NC] += prod[8 * i:8 * i + 8]
        first += n
    out_ref[0, :, D:] = jnp.concatenate(
        [jnp.sum(s, axis=0, keepdims=True) for s in sums], axis=1).astype(BF16)


def _cache_view(cache):
    assert cache.shape == (1, H, SK, DH)
    return jnp.swapaxes(cache, 2, 3).reshape(KV_BLOCKS, KV_ROWS, SK)


def _weight_view(w):
    tiles = w.reshape(w.shape[0] // 8, 8, w.shape[1] // T, T)
    return tiles.transpose(0, 2, 1, 3).reshape(W_BLOCKS, W_ROWS, T)


@jax.jit
def pallas_concat_heads__sliding_block_cached__sliding_block_cached__decode_kernel(
    A_x: jax.Array,
    A_k_cache: jax.Array,
    A_v_cache: jax.Array,
    A_wq: jax.Array,
    A_wo: jax.Array,
    B_x: jax.Array,
    B_k_cache: jax.Array,
    B_v_cache: jax.Array,
    B_wq: jax.Array,
    B_wo: jax.Array,
):
    return pl.pallas_call(
        _kernel,
        out_shape=jax.ShapeDtypeStruct((1, 1, 2 * D), BF16),
        in_specs=[pl.BlockSpec(memory_space=pltpu.HBM)] * 10,
        out_specs=pl.BlockSpec(memory_space=pltpu.VMEM),
        scratch_shapes=[
            pltpu.VMEM((2, 1, D), BF16),
            pltpu.VMEM((2 * KV_BLOCKS, KV_ROWS, W), BF16),
            pltpu.VMEM((2 * KV_BLOCKS, KV_ROWS, W), BF16),
            pltpu.VMEM((2 * W_BLOCKS, W_ROWS, T), BF16),
            pltpu.VMEM((2 * W_BLOCKS, W_ROWS, T), BF16),
            pltpu.VMEM((2, D // 8, T), F32),
            pltpu.VMEM((2, NT, T), F32),
            pltpu.VMEM((2, H // 8, 8, W), F32),
            pltpu.VMEM((2 * NT, T), F32),
            pltpu.VMEM((NC, 2 * NT, T), F32),
            pltpu.VMEM((sum(TAIL_VPU), T, T), F32),
            pltpu.SemaphoreType.DMA((SEM_TAIL + len(TAIL_VPU),)),
        ],
        compiler_params=pltpu.CompilerParams(
            vmem_limit_bytes=100 * 1024 * 1024,
            disable_bounds_checks=True,
            disable_semaphore_checks=True,
        ),
    )(
        A_x, _cache_view(A_k_cache), _cache_view(A_v_cache),
        _weight_view(A_wq), _weight_view(A_wo),
        B_x, _cache_view(B_k_cache), _cache_view(B_v_cache),
        _weight_view(B_wq), _weight_view(B_wo),
    )
```

```python
import jax
import jax.numpy as jnp
from jax import lax
import jax.experimental.pallas as pl
import jax.experimental.pallas.tpu as pltpu

BF16, F32 = jnp.bfloat16, jnp.float32

D, H, DH, SK = 640, 32, 192, 4096
W = min(4096, max(256, SK // 4))
T = 128
NT = H * DH // T
NC = D // T
GROUP = 8 * DH

KV_BLOCKS, KV_ROWS = 96, 64
W_BLOCKS, W_ROWS = 15, 2048
PIECE = 32

WQ, K, V, WO = 0, 2, 4, 6
ROUNDS = 64
LAG = 12
SETTLE = 8

STEPS = 16
TILES = NT // STEPS
TAIL_STEP = 26
TAIL_MXU = 8
TAIL_VPU = (3, 2, 1, 1)

SEM_X, SEM_WO = 10, 11
SEM_TAIL = SEM_WO + 2 * STEPS


def _loop(lo, hi, fn):
    lax.fori_loop(lo, hi, lambda i, carry: (fn(i), carry)[1], 0)


def _ds(start, size):
    if not isinstance(start, int):
        start = pl.multiple_of(start, size)
    return pl.ds(start, size)


def _iota(shape, axis):
    return lax.broadcasted_iota(jnp.int32, shape, axis)


def _ones_where(mask):
    return jnp.where(mask, 1.0, 0.0).astype(BF16)


def _kernel(a_x, a_k, a_v, a_wq, a_wo, b_x, b_k, b_v, b_wq, b_wo, out_ref,
            x_buf, k_buf, v_buf, wq_buf, wo_buf, x_rows, q_buf, p_buf, o_buf,
            o_rows, o_cols, sems):
    src = (a_wq, b_wq, a_k, b_k, a_v, b_v, a_wo, b_wo)
    dst = (wq_buf, wq_buf, k_buf, k_buf, v_buf, v_buf, wo_buf, wo_buf)

    def weight_copy(t, block, n, rows, sem):
        return pltpu.make_async_copy(
            src[t].at[pl.ds(block, n), rows],
            dst[t].at[pl.ds(t % 2 * W_BLOCKS + block, n), rows],
            sems.at[sem])

    def units(t):
        return 4 if K <= t < WO else 3

    def start_unit(t, rnd, unit, queue):
        if K <= t < WO:
            half = rnd >> 5
            rows = _ds((((rnd >> 1) & 6) | ((rnd >> 4) & 1)) * 8, 8)
            col = (unit >> 1) * (W // 2)
            block = half * 48 + (rnd & 3) * 12 + (unit & 1) * 6
            for first, n in ((1, 3), (4, 2)) if queue else ((0, 1),):
                pltpu.make_async_copy(
                    src[t].at[pl.ds(block + first, n), rows,
                              _ds(SK - W + col, W // 2)],
                    dst[t].at[pl.ds(t % 2 * KV_BLOCKS + block + first, n), rows,
                              _ds(col, W // 2)],
                    sems.at[2 * t - 2 + half]).start(priority=queue)
        else:
            rows = _ds(rnd * PIECE, PIECE)
            sem = t if t < K else SEM_WO + t % 2 * STEPS + (rnd >> 2)
            for first, n in ((1, 3), (4, 1)) if queue else ((0, 1),):
                weight_copy(t, 5 * unit + first, n, rows, sem).start(
                    priority=queue)

    def first_round(t, rnd):
        for unit in range(units(t)):
            if t and units(t) == units(t - 1):
                start_unit(t - 1, ROUNDS - LAG // units(t) + rnd, unit, 0)
            elif t:
                start_unit(t - 1, ROUNDS - units(t) + unit, rnd, 0)
            start_unit(t, rnd, unit, 1)

    def later_round(t, rnd):
        for unit in range(units(t)):
            start_unit(t, rnd - LAG // units(t), unit, 0)
            start_unit(t, rnd, unit, 1)

    def issue(lo, hi, first, last):
        clip_lo, clip_hi = ((max, min) if isinstance(first, int)
                            else (jnp.maximum, jnp.minimum))
        for t in range(len(src)):
            base, split = t * ROUNDS, LAG // units(t)
            for r0, r1, fn in ((0, split, first_round),
                               (split, ROUNDS, later_round)):
                if base + r1 > lo and base + r0 < hi:
                    _loop(clip_lo(first - base, r0), clip_hi(last - base, r1),
                          lambda rnd, fn=fn, t=t: fn(t, rnd))

    def issue_tail():
        copies = [(block, 2, _ds(W_ROWS - T + piece * PIECE, PIECE), SEM_TAIL - 1)
                  for piece in range(T // PIECE)
                  for block in range(0, TAIL_MXU, 2)]
        block = TAIL_MXU
        for batch, n in enumerate(TAIL_VPU):
            copies += [(block + i, 1, _ds(W_ROWS - T, T), SEM_TAIL + batch)
                       for i in range(n)]
            block += n
        for i in range(LAG):
            start_unit(WO + 1, ROUNDS - 8 + i // 3, i % 3, 0)
            for copy in copies[i * len(copies) // LAG:
                               (i + 1) * len(copies) // LAG]:
                weight_copy(WO + 1, *copy).start(priority=1)

    def wait(filled, sem):
        pltpu.make_async_copy(filled, filled, sems.at[sem]).wait()

    def stage(lo, hi, round_at, buf, parts, sem, compute):
        steps = 2 * STEPS // parts
        size = buf.shape[0] // parts

        def step(c):
            issue(lo, hi, round_at(c), round_at(c + 1))
            part = lax.div(c, steps)
            pl.when(lax.rem(c, steps) == 0)(
                lambda: wait(buf.at[pl.ds(part * size, size)], sem + part))
            compute(lax.div(c, STEPS), lax.rem(c, STEPS))

        _loop(0, 2 * STEPS, step)

    q_at = ROUNDS + SETTLE
    s_at = K * ROUNDS + ROUNDS // 2 + SETTLE
    o_at = V * ROUNDS + ROUNDS // 2 + SETTLE
    out_at = WO * ROUNDS + ROUNDS // 2 + SETTLE
    tail_at = len(src) * ROUNDS - 4

    first_round(WQ, 0)
    issue(1, ROUNDS, 1, ROUNDS)
    for br, x in enumerate((a_x, b_x)):
        pltpu.make_async_copy(x.at[0], x_buf.at[br], sems.at[SEM_X]).start()
    issue(ROUNDS, q_at, ROUNDS, q_at)
    q_buf[...] = jnp.zeros(q_buf.shape, F32)
    p_buf[...] = jnp.zeros(p_buf.shape, F32)
    wait(x_buf, SEM_X)

    def spread_x(br):
        own = (_iota((D // 8, D), 1) >> 3) == _iota((D // 8, D), 0)
        x = jnp.where(own, x_buf[br].astype(F32), 0.0).astype(BF16)
        spread = _ones_where((_iota((D, T), 0) & 7) == (_iota((D, T), 1) & 7))
        x_rows[br] = jnp.dot(x, spread, preferred_element_type=F32)

    _loop(0, 2, spread_x)

    def project_q(br, step):
        diagonal = (_iota((16, T), 1) >> 3) == _iota((16, T), 0)
        n = D // 8 // STEPS
        lhs, rhs = [], []
        for r in (step * n + i for i in range(n)):
            lhs.append(jnp.where(diagonal, x_rows[br, pl.ds(r, 1)], 0.0))
            rhs.append(jnp.concatenate(
                [wq_buf[br * W_BLOCKS + (u >> 4), _ds((u & 15) * T, T)]
                 for u in (3 * r, 3 * r + 1, 3 * r + 2)], axis=1))
        q = jnp.dot(jnp.concatenate(lhs, axis=1).astype(BF16),
                    jnp.concatenate(rhs, axis=0), preferred_element_type=F32)
        for i in range(3):
            q_buf[br, 16 * i:16 * (i + 1)] += q[:, i * T:(i + 1) * T]

    stage(q_at, s_at, lambda c: q_at + 4 * c - 2 * jnp.maximum(c - STEPS, 0),
          wq_buf, 2, 0, project_q)

    def own_head(step):
        row = _iota((8, TILES * T), 0)
        col = _iota((8, TILES * T), 1) + lax.rem(step * TILES * T, GROUP)
        return (col >= row * DH) & (col < (row + 1) * DH)

    def cache_rows(buf, br, step):
        n = KV_BLOCKS // STEPS
        return buf[pl.ds(br * KV_BLOCKS + step * n, n)].reshape(TILES * T, W)

    def scores(br, step):
        q = jnp.concatenate([q_buf[br, pl.ds(step * TILES + i, 1)]
                             for i in range(TILES)], axis=1)
        q = jnp.where(own_head(step), q, 0.0).astype(BF16)
        group = lax.div(step * TILES * T, GROUP)
        p_buf[br, group] += jnp.dot(q, cache_rows(k_buf, br, step),
                                    preferred_element_type=F32)

        @pl.when(lax.rem((step + 1) * TILES * T, GROUP) == 0)
        def _():
            s = p_buf[br, group] * (DH ** -0.5)
            e = jnp.exp(s - jnp.max(s, axis=-1, keepdims=True))
            p_buf[br, group] = e / jnp.sum(e, axis=-1, keepdims=True)

    stage(s_at, o_at, lambda c: s_at + 4 * c, k_buf, 4, 2, scores)

    def values(br, step):
        p = p_buf[br, lax.div(step * TILES * T, GROUP)].astype(BF16)
        o = lax.dot_general(p, cache_rows(v_buf, br, step),
                            (((1,), (1,)), ((), ())), preferred_element_type=F32)
        o = jnp.sum(jnp.where(own_head(step), o, 0.0), axis=0, keepdims=True)
        for i in range(TILES):
            o_buf[pl.ds(br * NT + step * TILES + i, 1)] = o[:, i * T:(i + 1) * T]

    stage(o_at, out_at, lambda c: o_at + 4 * c, v_buf, 4, 6, values)

    row, col = _iota((T, D), 0), _iota((T, D), 1)
    first = (row >> 3) * (8 * NC)
    spread = _ones_where((col >= first) & (col < first + 8 * NC)
                         & ((col & 7) == (row & 7)))
    o = jnp.dot(o_buf[...].astype(BF16), spread, preferred_element_type=F32)
    for i in range(NC):
        o_rows[i] = o[:, i * T:(i + 1) * T]

    row = _iota((8, T), 0)
    phase = row - (_iota((8, T), 1) >> 3) + 3 * NC
    for _ in range(3):
        phase = jnp.where(phase >= NC, phase - NC, phase)
    phase = jnp.where(row < NC, phase, -1)

    def project_out(acc, br, group, blocks, sem):
        lhs = [None] * blocks
        for i in range(NC):
            u = i * STEPS + group
            plane, r = lax.rem(u, NC), br * NT + lax.div(u, NC)
            for block in range(i, blocks, NC):
                o = o_rows[plane, pl.ds(r + block // NC * STEPS, 1)]
                lhs[block] = jnp.where(phase == plane, o, 0.0)
        lhs = jnp.concatenate(lhs, axis=1).astype(BF16)
        wo = wo_buf.at[pl.ds(br * W_BLOCKS, blocks), _ds(group * T, T)]
        wait(wo, sem)
        return acc + jnp.dot(lhs, wo[...].reshape(blocks * T, T),
                             preferred_element_type=F32)

    def out_step(c, acc):
        rate = pl.cdiv((tail_at - out_at) * 16, TAIL_STEP)
        issue(out_at, tail_at,
              jnp.minimum(out_at + ((c * rate) >> 4), tail_at),
              jnp.minimum(out_at + (((c + 1) * rate) >> 4), tail_at))
        pl.when(c == TAIL_STEP)(issue_tail)

        @pl.when(c < sum(TAIL_VPU))
        def _():
            u = (TAIL_MXU + c + 1) * STEPS - 1
            o = o_rows[lax.rem(u, NC), pl.ds(NT + lax.div(u, NC), 1)]
            o_cols[c] = jnp.broadcast_to(o, (T, T)).T

        @pl.when(c == STEPS)
        def _():
            out_ref[0, :, :D] = jnp.concatenate(
                [acc[i:i + 1] for i in range(NC)], axis=1).astype(BF16)

        return project_out(jnp.where(c == STEPS, 0.0, acc), lax.div(c, STEPS),
                           lax.rem(c, STEPS), W_BLOCKS, SEM_WO + c)

    acc = lax.fori_loop(0, 2 * STEPS - 1, out_step, jnp.zeros((8, T), F32))
    acc = project_out(acc, 1, STEPS - 1, TAIL_MXU, SEM_TAIL - 1)

    sums = [jnp.where(row == i, acc, 0.0) for i in range(NC)]
    first = TAIL_MXU
    for batch, n in enumerate(TAIL_VPU):
        wait(wo_buf.at[pl.ds(W_BLOCKS + first, n), _ds(W_ROWS - T, T)],
             SEM_TAIL + batch)
        for block in range(first, first + n):
            prod = (wo_buf[W_BLOCKS + block, W_ROWS - T:].astype(F32)
                    * o_cols[block - TAIL_MXU])
            for i in range(T // 8):
                sums[((block + 1) * STEPS - 1 + i) % NC] += prod[8 * i:8 * i + 8]
        first += n
    out_ref[0, :, D:] = jnp.concatenate(
        [jnp.sum(s, axis=0, keepdims=True) for s in sums], axis=1).astype(BF16)


def _cache_view(cache):
    assert cache.shape == (1, H, SK, DH)
    return jnp.swapaxes(cache, 2, 3).reshape(KV_BLOCKS, KV_ROWS, SK)


def _weight_view(w):
    tiles = w.reshape(w.shape[0] // 8, 8, w.shape[1] // T, T)
    return tiles.transpose(0, 2, 1, 3).reshape(W_BLOCKS, W_ROWS, T)


@jax.jit
def pallas_concat_heads__sliding_block_cached__sliding_block_cached__decode_kernel(
    A_x: jax.Array,
    A_k_cache: jax.Array,
    A_v_cache: jax.Array,
    A_wq: jax.Array,
    A_wo: jax.Array,
    B_x: jax.Array,
    B_k_cache: jax.Array,
    B_v_cache: jax.Array,
    B_wq: jax.Array,
    B_wo: jax.Array,
):
    return pl.pallas_call(
        _kernel,
        out_shape=jax.ShapeDtypeStruct((1, 1, 2 * D), BF16),
        in_specs=[pl.BlockSpec(memory_space=pltpu.HBM)] * 10,
        out_specs=pl.BlockSpec(memory_space=pltpu.VMEM),
        scratch_shapes=[
            pltpu.VMEM((2, 1, D), BF16),
            pltpu.VMEM((2 * KV_BLOCKS, KV_ROWS, W), BF16),
            pltpu.VMEM((2 * KV_BLOCKS, KV_ROWS, W), BF16),
            pltpu.VMEM((2 * W_BLOCKS, W_ROWS, T), BF16),
            pltpu.VMEM((2 * W_BLOCKS, W_ROWS, T), BF16),
            pltpu.VMEM((2, D // 8, T), F32),
            pltpu.VMEM((2, NT, T), F32),
            pltpu.VMEM((2, H // 8, 8, W), F32),
            pltpu.VMEM((2 * NT, T), F32),
            pltpu.VMEM((NC, 2 * NT, T), F32),
            pltpu.VMEM((sum(TAIL_VPU), T, T), F32),
            pltpu.SemaphoreType.DMA((SEM_TAIL + len(TAIL_VPU),)),
        ],
        compiler_params=pltpu.CompilerParams(
            vmem_limit_bytes=100 * 1024 * 1024,
            disable_bounds_checks=True,
            disable_semaphore_checks=True,
        ),
    )(
        A_x, _cache_view(A_k_cache), _cache_view(A_v_cache),
        _weight_view(A_wq), _weight_view(A_wo),
        B_x, _cache_view(B_k_cache), _cache_view(B_v_cache),
        _weight_view(B_wq), _weight_view(B_wo),
    )
```
